```python
import os as _os
_os.environ.setdefault("JAX_PLATFORMS", "cpu")
import jax
import jax.numpy as jnp

def _softmax(x, axis=-1):
    return jax.nn.softmax(x, axis=axis)
def _gelu(x):
    return jax.nn.gelu(x, approximate=True)
def _silu(x):
    return jax.nn.silu(x)
def _sigmoid(x):
    return jax.nn.sigmoid(x)
def _layernorm(x, axis=-1, eps=1e-5):
    m = jnp.mean(x, axis=axis, keepdims=True)
    v = jnp.var(x, axis=axis, keepdims=True)
    return (x - m) / jnp.sqrt(v + eps)
def _scatter_add(tgt, idx, src, axis=0):
    return tgt.at[idx].add(src)
def _segment_sum(src, seg, n):
    return jax.ops.segment_sum(src, seg, n)
class _Rng:
    def __init__(self, key):
        self._k = key
    def _next(self):
        self._k, sub = jax.random.split(self._k)
        return sub
    def normal(self, shape):
        return jax.random.normal(self._next(), shape, dtype=jnp.bfloat16)
    def randint(self, lo, hi, shape):
        return jax.random.randint(self._next(), shape, lo, hi, dtype=jnp.int32)
    def uniform(self, shape, lo=0.0, hi=1.0):
        return jax.random.uniform(self._next(), shape, jnp.bfloat16, lo, hi)
    def permutation(self, n):
        return jax.random.permutation(self._next(), n)


kernel_name = 'concat_heads__grouped_kv_mqa__sliding_block__prompt'

def setup_inputs():
    _rng = _Rng(jax.random.key(int.from_bytes(__import__("os").urandom(4), "little")))
    _w = (lambda a: (lambda t: t.astype(jnp.bfloat16) if jnp.issubdtype(t.dtype, jnp.floating) else t)(jnp.asarray(a)))
    def _A_setup():
        B, S, D, H = 1, 2048, 1024, 32
        Dh = D // H
        return {
            "x": _w((lambda *s: _rng.normal(s) * 0.05)(B, S, D)),
            "wq": _w((lambda *s: _rng.normal(s) * 1.6)(D, H * Dh)),
            "wk": _w((lambda *s: _rng.normal(s) * 1.6)(D, Dh)),
            "wv": _w((lambda *s: _rng.normal(s) * 0.1)(D, Dh)),
            "wo": _w((lambda *s: _rng.normal(s) * 0.1)(H * Dh, D)),
        }
    _A_in = _A_setup()

    def _B_setup():
        B, S, D = 1, 2048, 1024
        return {
            "x": _w((lambda *s: _rng.normal(s) * 0.2)(B, S, D)),
            "wqkv": _w((lambda *s: _rng.normal(s) * 0.2)(D, 3 * D)),
            "wo": _w((lambda *s: _rng.normal(s) * 0.05)(D, D)),
        }
    _B_in = _B_setup()

    return {
        "A_x": _A_in["x"],
        "A_wq": _A_in["wq"],
        "A_wk": _A_in["wk"],
        "A_wv": _A_in["wv"],
        "A_wo": _A_in["wo"],
        "B_x": _B_in["x"],
        "B_wqkv": _B_in["wqkv"],
        "B_wo": _B_in["wo"],
    }

def reference(A_x, A_wq, A_wk, A_wv, A_wo, B_x, B_wqkv, B_wo):
    def _A_ref(x, wq, wk, wv, wo):
        B, S, D = x.shape
        H = 32
        Dh = D // H
        q = (lambda x, *d: x.transpose(*d))((x @ wq).reshape(B, S, H, Dh), 0, 2, 1, 3)
        k = x @ wk
        v = x @ wv
        scores = jnp.einsum("bhqd,bkd->bhqk", q, k) * (Dh ** -0.5)
        p = _softmax(scores, axis=-1)
        o = jnp.einsum("bhqk,bkd->bhqd", p, v)
        return (lambda x, *d: x.transpose(*d))(o, 0, 2, 1, 3).reshape(B, S, H * Dh) @ wo

    def _B_ref(x, wqkv, wo):
        B, S, D = x.shape
        H = 32; Dh = D // H; W = 256
        qkv = (lambda x, *d: x.transpose(*d))((x @ wqkv).reshape(B, S, 3, H, Dh), 2, 0, 3, 1, 4)
        q, k, v = qkv[0], qkv[1], qkv[2]
        scores = jnp.einsum("bhqd,bhkd->bhqk", q, k) * (Dh ** -0.5)
        idx = jnp.arange(S)
        mask = (idx[:, None] - idx[None, :] >= 0) & (idx[:, None] - idx[None, :] < W)
        scores = jnp.where(mask[None, None], scores, -1e9)
        p = _softmax(scores, axis=-1)
        o = jnp.einsum("bhqk,bhkd->bhqd", p, v)
        return (lambda x, *d: x.transpose(*d))(o, 0, 2, 1, 3).reshape(B, S, D) @ wo

    a = _A_ref(A_x, A_wq, A_wk, A_wv, A_wo)
    b = _B_ref(B_x, B_wqkv, B_wo)
    return jnp.concatenate([a, b], axis=-1)
```

```python
import functools
import jax
import jax.numpy as jnp
from jax import lax
import jax.experimental.pallas as pl
import jax.experimental.pallas.tpu as pltpu

S = 2048
D = 1024
H = 32
DH = 32
W = 256
TQ = 256
NT = S // TQ
LOG2E = 1.4426950408889634
QSCALE = (DH ** -0.5) * LOG2E
CK = 256
NC = S // CK
KW = 384
NSUB = TQ // 128
NEG = -1e30


def _kernel(xa_ref, wq_ref, wk_ref, wv_ref, woa_ref, xb_ref, wqkv_ref, wob_ref,
            o_ref,
            ka_ref, vta_ref, qt_ref, ot_ref, kb_ref, vtb_ref, sa0, sa1, qm_ref, bias_ref,
            sb0, sb1):
    t = pl.program_id(0)
    f32 = jnp.float32
    bf16 = jnp.bfloat16

    @pl.when(t == 0)
    def _init():
        xa = xa_ref[...]
        k = jnp.dot(xa, wk_ref[...], preferred_element_type=f32)
        v = jnp.dot(xa, wv_ref[...], preferred_element_type=f32)
        ka_ref[...] = k.astype(bf16)
        vta_ref[...] = v.T.astype(bf16)
        kb_ref[...] = jnp.zeros(kb_ref.shape, bf16)
        vtb_ref[...] = jnp.zeros(vtb_ref.shape, bf16)

    row0 = pl.multiple_of(t * TQ, TQ)

    xa_t = xa_ref[pl.ds(row0, TQ), :]
    q = jnp.dot(xa_t, wq_ref[...], preferred_element_type=f32) * QSCALE
    qt_ref[...] = q.T.astype(bf16)

    def qk_a(h, buf):
        r0 = pl.multiple_of(h * DH, DH)
        qh = qt_ref[pl.ds(r0, DH), :]
        m8 = None
        for c in range(NC):
            st = jnp.dot(ka_ref[c * CK:(c + 1) * CK, :], qh, preferred_element_type=f32)
            buf[c * CK:(c + 1) * CK, :] = st
            mc = jnp.max(st.reshape(CK // 8, 8, TQ), axis=0)
            m8 = mc if m8 is None else jnp.maximum(m8, mc)
        return jnp.max(m8, axis=0, keepdims=True)

    def pv_a(h, buf, m):
        r0 = pl.multiple_of(h * DH, DH)
        l8 = None
        acc = None
        for c in range(NC):
            p = jnp.exp2(buf[c * CK:(c + 1) * CK, :] - m)
            lc = jnp.sum(p.reshape(CK // 8, 8, TQ), axis=0)
            l8 = lc if l8 is None else l8 + lc
            d = jnp.dot(vta_ref[:, c * CK:(c + 1) * CK], p.astype(bf16),
                        preferred_element_type=f32)
            acc = d if acc is None else acc + d
        ot_ref[pl.ds(r0, DH), :] = acc / jnp.sum(l8, axis=0, keepdims=True)

    def body_a(i, m):
        h = 2 * i
        m1 = qk_a(h + 1, sa1)
        pv_a(h, sa0, m)
        m2 = qk_a(jnp.minimum(h + 2, H - 1), sa0)
        pv_a(h + 1, sa1, m1)
        return m2

    with jax.named_scope("attnA"):
        lax.fori_loop(0, H // 2, body_a, qk_a(0, sa0))
    oa = ot_ref[...].T.astype(bf16)
    o_ref[:, 0:D] = jnp.dot(oa, woa_ref[...], preferred_element_type=f32).astype(o_ref.dtype)

    xb_t = xb_ref[...]
    qb = jnp.dot(xb_t, wqkv_ref[:, 0:D], preferred_element_type=f32) * QSCALE
    qbt = qb.T
    rowj = (lax.broadcasted_iota(jnp.int32, (D, TQ), 0) // DH) % 4
    for j in range(4):
        qm_ref[j] = jnp.where(rowj == j, qbt, 0.0).astype(bf16)
    kb = jnp.dot(xb_t, wqkv_ref[:, D:2 * D], preferred_element_type=f32)
    kb_ref[pl.ds(row0, TQ), :] = kb.astype(bf16)
    vb = jnp.dot(xb_t, wqkv_ref[:, 2 * D:3 * D], preferred_element_type=f32)
    vtb_ref[:, pl.ds(row0, TQ)] = vb.T.astype(bf16)

    k0s = []
    for sub in range(NSUB):
        q0 = row0 + sub * 128
        k0 = pl.multiple_of(jnp.maximum(q0 - 256, 0), 128)
        k0s.append(k0)
        kpos = k0 + lax.broadcasted_iota(jnp.int32, (KW, 128), 0)
        qpos = q0 + lax.broadcasted_iota(jnp.int32, (KW, 128), 1)
        d = qpos - kpos
        bias_ref[sub] = jnp.where((d >= 0) & (d < W), 0.0, NEG).astype(f32)

    def qk_b(g, buf):
        c0 = pl.multiple_of(g * 128, 128)
        ms = []
        for sub in range(NSUB):
            kg = kb_ref[pl.ds(k0s[sub], KW), pl.ds(c0, 128)]
            for j in range(4):
                qm = qm_ref[j, pl.ds(c0, 128), sub * 128:(sub + 1) * 128]
                st = jnp.dot(kg, qm, preferred_element_type=f32) + bias_ref[sub]
                buf[sub * 4 + j] = st
                ms.append(jnp.max(st, axis=0, keepdims=True))
        return tuple(ms)

    def pv_b(g, buf, ms):
        c0 = pl.multiple_of(g * 128, 128)
        for sub in range(NSUB):
            vtg = vtb_ref[pl.ds(c0, 128), pl.ds(k0s[sub], KW)]
            for j in range(4):
                p = jnp.exp2(buf[sub * 4 + j] - ms[sub * 4 + j])
                l = jnp.sum(p, axis=0, keepdims=True)
                ot = jnp.dot(vtg[j * DH:(j + 1) * DH, :], p.astype(bf16),
                             preferred_element_type=f32)
                ot_ref[pl.ds(c0 + j * DH, DH), sub * 128:(sub + 1) * 128] = ot / l

    def body_b(i, ms):
        g = 2 * i
        ms1 = qk_b(g + 1, sb1)
        pv_b(g, sb0, ms)
        ms2 = qk_b(jnp.minimum(g + 2, H // 4 - 1), sb0)
        pv_b(g + 1, sb1, ms1)
        return ms2

    with jax.named_scope("attnB"):
        lax.fori_loop(0, H // 8, body_b, qk_b(0, sb0))

    ob = ot_ref[...].T.astype(bf16)
    o_ref[:, D:2 * D] = jnp.dot(ob, wob_ref[...], preferred_element_type=f32).astype(o_ref.dtype)


@jax.jit
def pallas_concat_heads__grouped_kv_mqa__sliding_block__prompt_kernel(A_x, A_wq, A_wk, A_wv, A_wo, B_x, B_wqkv, B_wo):
    xa = A_x.reshape(S, D)
    xb = B_x.reshape(S, D)
    bf16 = jnp.bfloat16
    f32 = jnp.float32
    const = lambda shape: pl.BlockSpec(shape, lambda t: (0, 0))
    out = pl.pallas_call(
        _kernel,
        grid=(NT,),
        in_specs=[
            const((S, D)), const((D, D)), const((D, DH)), const((D, DH)), const((D, D)),
            pl.BlockSpec((TQ, D), lambda t: (t, 0)), const((D, 3 * D)), const((D, D)),
        ],
        out_specs=pl.BlockSpec((TQ, 2 * D), lambda t: (t, 0)),
        out_shape=jax.ShapeDtypeStruct((S, 2 * D), bf16),
        scratch_shapes=[
            pltpu.VMEM((S, DH), bf16),
            pltpu.VMEM((DH, S), bf16),
            pltpu.VMEM((D, TQ), bf16),
            pltpu.VMEM((D, TQ), f32),
            pltpu.VMEM((S, D), bf16),
            pltpu.VMEM((D, S), bf16),
            pltpu.VMEM((S, TQ), f32),
            pltpu.VMEM((S, TQ), f32),
            pltpu.VMEM((4, D, TQ), bf16),
            pltpu.VMEM((NSUB, KW, 128), f32),
            pltpu.VMEM((NSUB * 4, KW, 128), f32),
            pltpu.VMEM((NSUB * 4, KW, 128), f32),
        ],
        compiler_params=pltpu.CompilerParams(
            dimension_semantics=("arbitrary",),
            vmem_limit_bytes=100 * 1024 * 1024),
    )(xa, A_wq, A_wk, A_wv, A_wo, xb, B_wqkv, B_wo)
    return out.reshape(1, S, 2 * D)
```

```python
import jax
import jax.numpy as jnp
from jax import lax
import jax.experimental.pallas as pl
import jax.experimental.pallas.tpu as pltpu

S = 2048
D = 1024
H = 32
DH = 32
W = 256
TQ = 256
NT = S // TQ
LOG2E = 1.4426950408889634
QSCALE = (DH ** -0.5) * LOG2E
CK = 256
NC = S // CK
KW = 384
NSUB = TQ // 128
NG = H // 4
NEG = -1e30


def _kernel(xa_hbm, wq_hbm, wkt_ref, wvt_ref, woa_hbm, xb_ref, wqkv_hbm, wob_hbm,
            o_ref,
            xa_ref, wq_ref, woa_ref, wqkv_ref, wob_ref, sems,
            ka_ref, vta_ref, qt_ref, ota_ref, otb_ref, kb_ref, vtb_ref, sa0, sa1, qm_ref,
            bias_ref, sb0, sb1):
    t = pl.program_id(0)
    f32 = jnp.float32
    bf16 = jnp.bfloat16

    copies = [
        pltpu.make_async_copy(wqkv_hbm.at[:, 0:D], wqkv_ref.at[:, 0:D], sems.at[0]),
        pltpu.make_async_copy(wqkv_hbm.at[:, D:2 * D], wqkv_ref.at[:, D:2 * D], sems.at[1]),
        pltpu.make_async_copy(wqkv_hbm.at[:, 2 * D:3 * D], wqkv_ref.at[:, 2 * D:3 * D], sems.at[2]),
        pltpu.make_async_copy(xa_hbm, xa_ref, sems.at[3]),
        pltpu.make_async_copy(wq_hbm, wq_ref, sems.at[4]),
        pltpu.make_async_copy(wob_hbm, wob_ref, sems.at[5]),
        pltpu.make_async_copy(woa_hbm, woa_ref, sems.at[6]),
    ]

    def wait(i):
        @pl.when(t == 0)
        def _():
            copies[i].wait()

    @pl.when(t == 0)
    def _start():
        for c in copies:
            c.start()
        kb_ref[TQ:KW, :] = jnp.zeros((KW - TQ, D), bf16)
        vtb_ref[:, TQ:KW] = jnp.zeros((D, KW - TQ), bf16)

    row0 = pl.multiple_of(t * TQ, TQ)

    xb_t = xb_ref[...]
    wait(0)
    qb = jnp.dot(xb_t, wqkv_ref[:, 0:D], preferred_element_type=f32) * QSCALE
    qbt = qb.T
    rowj = (lax.broadcasted_iota(jnp.int32, (D, TQ), 0) // DH) % 4
    for j in range(4):
        qm_ref[j] = jnp.where(rowj == j, qbt, 0.0).astype(bf16)
    wait(1)
    kb = jnp.dot(xb_t, wqkv_ref[:, D:2 * D], preferred_element_type=f32)
    kb_ref[pl.ds(row0, TQ), :] = kb.astype(bf16)
    wait(2)
    vb = jnp.dot(xb_t, wqkv_ref[:, 2 * D:3 * D], preferred_element_type=f32)
    vtb_ref[:, pl.ds(row0, TQ)] = vb.T.astype(bf16)

    k0s = []
    for sub in range(NSUB):
        q0 = row0 + sub * 128
        k0 = pl.multiple_of(jnp.maximum(q0 - W, 0), 128)
        k0s.append(k0)
        kpos = k0 + lax.broadcasted_iota(jnp.int32, (KW, 128), 0)
        qpos = q0 + lax.broadcasted_iota(jnp.int32, (KW, 128), 1)
        d = qpos - kpos
        bias_ref[sub] = jnp.where((d >= 0) & (d < W), 0.0, NEG).astype(f32)

    def qk_b(g, buf):
        c0 = pl.multiple_of(g * 128, 128)
        ms = []
        for sub in range(NSUB):
            kg = kb_ref[pl.ds(k0s[sub], KW), pl.ds(c0, 128)]
            for j in range(4):
                qm = qm_ref[j, pl.ds(c0, 128), sub * 128:(sub + 1) * 128]
                st = jnp.dot(kg, qm, preferred_element_type=f32) + bias_ref[sub]
                buf[sub * 4 + j] = st
                ms.append(jnp.max(st, axis=0, keepdims=True))
        return tuple(ms)

    def pv_b(g, buf, ms):
        c0 = pl.multiple_of(g * 128, 128)
        for sub in range(NSUB):
            vtg = vtb_ref[pl.ds(c0, 128), pl.ds(k0s[sub], KW)]
            for j in range(4):
                p = jnp.exp2(buf[sub * 4 + j] - ms[sub * 4 + j])
                l = jnp.sum(p, axis=0, keepdims=True)
                ot = jnp.dot(vtg[j * DH:(j + 1) * DH, :], p.astype(bf16),
                             preferred_element_type=f32)
                otb_ref[pl.ds(c0 + j * DH, DH), sub * 128:(sub + 1) * 128] = ot / l

    def body_b(i, ms):
        g = 2 * i
        ms1 = qk_b(g + 1, sb1)
        pv_b(g, sb0, ms)
        ms2 = qk_b(g + 2, sb0)
        pv_b(g + 1, sb1, ms1)
        return ms2

    ms = lax.fori_loop(0, NG // 2 - 1, body_b, qk_b(0, sb0))

    @pl.when(t == 0)
    def _init_kv_a():
        copies[3].wait()
        xa = xa_ref[...]
        nt = (((1,), (1,)), ((), ()))
        k = lax.dot_general(xa, wkt_ref[...], nt, preferred_element_type=f32)
        vt = lax.dot_general(wvt_ref[...], xa, nt, preferred_element_type=f32)
        ka_ref[...] = k.astype(bf16)
        vta_ref[...] = vt.astype(bf16)
        copies[4].wait()

    ms1 = qk_b(NG - 1, sb1)
    pv_b(NG - 2, sb0, ms)
    pv_b(NG - 1, sb1, ms1)

    xa_t = xa_ref[pl.ds(row0, TQ), :]
    q = jnp.dot(xa_t, wq_ref[...], preferred_element_type=f32) * QSCALE
    qt_ref[...] = q.T.astype(bf16)

    def qk_a(h, buf):
        r0 = pl.multiple_of(h * DH, DH)
        qh = qt_ref[pl.ds(r0, DH), :]
        m8 = None
        for c in range(NC):
            st = jnp.dot(ka_ref[c * CK:(c + 1) * CK, :], qh, preferred_element_type=f32)
            buf[c * CK:(c + 1) * CK, :] = st
            mc = jnp.max(st.reshape(CK // 8, 8, TQ), axis=0)
            m8 = mc if m8 is None else jnp.maximum(m8, mc)
        return jnp.max(m8, axis=0, keepdims=True)

    def pv_a(h, buf, m):
        r0 = pl.multiple_of(h * DH, DH)
        l8 = None
        acc = None
        for c in range(NC):
            p = jnp.exp2(buf[c * CK:(c + 1) * CK, :] - m)
            lc = jnp.sum(p.reshape(CK // 8, 8, TQ), axis=0)
            l8 = lc if l8 is None else l8 + lc
            d = jnp.dot(vta_ref[:, c * CK:(c + 1) * CK], p.astype(bf16),
                        preferred_element_type=f32)
            acc = d if acc is None else acc + d
        ota_ref[pl.ds(r0, DH), :] = acc / jnp.sum(l8, axis=0, keepdims=True)

    def body_a(i, m):
        h = 2 * i
        m1 = qk_a(h + 1, sa1)
        pv_a(h, sa0, m)
        m2 = qk_a(h + 2, sa0)
        pv_a(h + 1, sa1, m1)
        return m2

    m = lax.fori_loop(0, H // 2 - 1, body_a, qk_a(0, sa0))

    @pl.when(t == 0)
    def _wait_wo():
        copies[5].wait()
        copies[6].wait()

    m1 = qk_a(H - 1, sa1)
    pv_a(H - 2, sa0, m)
    pv_a(H - 1, sa1, m1)

    ob = otb_ref[...].T.astype(bf16)
    o_ref[:, D:2 * D] = jnp.dot(ob, wob_ref[...], preferred_element_type=f32).astype(o_ref.dtype)
    oa = ota_ref[...].T.astype(bf16)
    o_ref[:, 0:D] = jnp.dot(oa, woa_ref[...], preferred_element_type=f32).astype(o_ref.dtype)


@jax.jit
def pallas_concat_heads__grouped_kv_mqa__sliding_block__prompt_kernel(
    A_x: jax.Array,
    A_wq: jax.Array,
    A_wk: jax.Array,
    A_wv: jax.Array,
    A_wo: jax.Array,
    B_x: jax.Array,
    B_wqkv: jax.Array,
    B_wo: jax.Array,
):
    xa = A_x.reshape(S, D)
    xb = B_x.reshape(S, D)
    bf16 = jnp.bfloat16
    f32 = jnp.float32
    const = lambda shape: pl.BlockSpec(shape, lambda t: (0, 0))
    hbm = pl.BlockSpec(memory_space=pl.ANY)
    out = pl.pallas_call(
        _kernel,
        grid=(NT,),
        in_specs=[
            hbm, hbm, const((DH, D)), const((DH, D)), hbm,
            pl.BlockSpec((TQ, D), lambda t: (t, 0)), hbm, hbm,
        ],
        out_specs=pl.BlockSpec((TQ, 2 * D), lambda t: (t, 0)),
        out_shape=jax.ShapeDtypeStruct((S, 2 * D), bf16),
        scratch_shapes=[
            pltpu.VMEM((S, D), bf16),
            pltpu.VMEM((D, D), bf16),
            pltpu.VMEM((D, D), bf16),
            pltpu.VMEM((D, 3 * D), bf16),
            pltpu.VMEM((D, D), bf16),
            pltpu.SemaphoreType.DMA((7,)),
            pltpu.VMEM((S, DH), bf16),
            pltpu.VMEM((DH, S), bf16),
            pltpu.VMEM((D, TQ), bf16),
            pltpu.VMEM((D, TQ), f32),
            pltpu.VMEM((D, TQ), f32),
            pltpu.VMEM((S, D), bf16),
            pltpu.VMEM((D, S), bf16),
            pltpu.VMEM((S, TQ), f32),
            pltpu.VMEM((S, TQ), f32),
            pltpu.VMEM((4, D, TQ), bf16),
            pltpu.VMEM((NSUB, KW, 128), f32),
            pltpu.VMEM((NSUB * 4, KW, 128), f32),
            pltpu.VMEM((NSUB * 4, KW, 128), f32),
        ],
        compiler_params=pltpu.CompilerParams(
            dimension_semantics=("arbitrary",),
            vmem_limit_bytes=100 * 1024 * 1024),
    )(xa, A_wq, A_wk.T, A_wv.T, A_wo, xb, B_wqkv, B_wo)
    return out.reshape(1, S, 2 * D)
```

```python
import jax
import jax.numpy as jnp
from jax import lax
import jax.experimental.pallas as pl
import jax.experimental.pallas.tpu as pltpu

S = 2048
D = 1024
H = 32
DH = 32
W = 256
TQ = 256
NT = S // TQ
LOG2E = 1.4426950408889634
QSCALE = (DH ** -0.5) * LOG2E
CK = 256
NC = S // CK
CQ = 256
KW = 384
NSUB = TQ // 128
NG = H // 4
NEG = -1e30


def _kernel(xa_hbm, wq_hbm, wkt_ref, wvt_ref, woa_hbm, xb_ref, wqkv_hbm, wob_hbm,
            o_ref,
            xa_ref, wq_ref, woa_ref, wqkv_ref, wob_ref, sems,
            ka_ref, vta_ref, qt_ref, ota_ref, otb_ref, kb_ref, vtb_ref, sa0, sa1, qm_ref,
            bias_ref, sb0, sb1):
    t = pl.program_id(0)
    f32 = jnp.float32
    bf16 = jnp.bfloat16

    copies = [
        pltpu.make_async_copy(wqkv_hbm.at[:, 0:D], wqkv_ref.at[:, 0:D], sems.at[0]),
        pltpu.make_async_copy(wqkv_hbm.at[:, D:2 * D], wqkv_ref.at[:, D:2 * D], sems.at[1]),
        pltpu.make_async_copy(wqkv_hbm.at[:, 2 * D:3 * D], wqkv_ref.at[:, 2 * D:3 * D], sems.at[2]),
        pltpu.make_async_copy(xa_hbm, xa_ref, sems.at[3]),
        pltpu.make_async_copy(wq_hbm, wq_ref, sems.at[4]),
        pltpu.make_async_copy(wob_hbm, wob_ref, sems.at[5]),
        pltpu.make_async_copy(woa_hbm, woa_ref, sems.at[6]),
    ]

    def wait(i):
        @pl.when(t == 0)
        def _():
            copies[i].wait()

    @pl.when(t == 0)
    def _start():
        for c in copies:
            c.start()
        kb_ref[TQ:KW, :] = jnp.zeros((KW - TQ, D), bf16)
        vtb_ref[:, TQ:KW] = jnp.zeros((D, KW - TQ), bf16)

    row0 = pl.multiple_of(t * TQ, TQ)

    xb_t = xb_ref[...]
    wait(0)
    qb = jnp.dot(xb_t, wqkv_ref[:, 0:D], preferred_element_type=f32) * QSCALE
    qbt = qb.T
    rowj = (lax.broadcasted_iota(jnp.int32, (D, TQ), 0) // DH) % 4
    for j in range(4):
        qm_ref[j] = jnp.where(rowj == j, qbt, 0.0).astype(bf16)
    wait(1)
    kb = jnp.dot(xb_t, wqkv_ref[:, D:2 * D], preferred_element_type=f32)
    kb_ref[pl.ds(row0, TQ), :] = kb.astype(bf16)
    wait(2)
    vb = jnp.dot(xb_t, wqkv_ref[:, 2 * D:3 * D], preferred_element_type=f32)
    vtb_ref[:, pl.ds(row0, TQ)] = vb.T.astype(bf16)

    k0s = []
    for sub in range(NSUB):
        q0 = row0 + sub * 128
        k0 = pl.multiple_of(jnp.maximum(q0 - W, 0), 128)
        k0s.append(k0)
        kpos = k0 + lax.broadcasted_iota(jnp.int32, (KW, 128), 0)
        qpos = q0 + lax.broadcasted_iota(jnp.int32, (KW, 128), 1)
        d = qpos - kpos
        bias_ref[sub] = jnp.where((d >= 0) & (d < W), 0.0, NEG).astype(f32)

    def qk_b(g, buf):
        c0 = pl.multiple_of(g * 128, 128)
        ms = []
        for sub in range(NSUB):
            kg = kb_ref[pl.ds(k0s[sub], KW), pl.ds(c0, 128)]
            for j in range(4):
                qm = qm_ref[j, pl.ds(c0, 128), sub * 128:(sub + 1) * 128]
                st = jnp.dot(kg, qm, preferred_element_type=f32) + bias_ref[sub]
                buf[sub * 4 + j] = st
                ms.append(jnp.max(st, axis=0, keepdims=True))
        return tuple(ms)

    def pv_b(g, buf, ms):
        c0 = pl.multiple_of(g * 128, 128)
        for sub in range(NSUB):
            vtg = vtb_ref[pl.ds(c0, 128), pl.ds(k0s[sub], KW)]
            for j in range(4):
                p = jnp.exp2(buf[sub * 4 + j] - ms[sub * 4 + j])
                l = jnp.sum(p, axis=0, keepdims=True)
                ot = jnp.dot(vtg[j * DH:(j + 1) * DH, :], p.astype(bf16),
                             preferred_element_type=f32)
                otb_ref[pl.ds(c0 + j * DH, DH), sub * 128:(sub + 1) * 128] = ot / l

    def stage_b(gq, bufq, gp, bufp, msp):
        cq = pl.multiple_of(gq * 128, 128)
        cp = pl.multiple_of(gp * 128, 128)
        ms = []
        for sub in range(NSUB):
            kg = kb_ref[pl.ds(k0s[sub], KW), pl.ds(cq, 128)]
            vtg = vtb_ref[pl.ds(cp, 128), pl.ds(k0s[sub], KW)]
            for j in range(4):
                qm = qm_ref[j, pl.ds(cq, 128), sub * 128:(sub + 1) * 128]
                st = jnp.dot(kg, qm, preferred_element_type=f32) + bias_ref[sub]
                bufq[sub * 4 + j] = st
                ms.append(jnp.max(st, axis=0, keepdims=True))
                p = jnp.exp2(bufp[sub * 4 + j] - msp[sub * 4 + j])
                l = jnp.sum(p, axis=0, keepdims=True)
                ot = jnp.dot(vtg[j * DH:(j + 1) * DH, :], p.astype(bf16),
                             preferred_element_type=f32)
                otb_ref[pl.ds(cp + j * DH, DH), sub * 128:(sub + 1) * 128] = ot / l
        return tuple(ms)

    def body_b(i, ms):
        g = 2 * i
        ms1 = stage_b(g + 1, sb1, g, sb0, ms)
        return stage_b(g + 2, sb0, g + 1, sb1, ms1)

    ms = lax.fori_loop(0, NG // 2 - 1, body_b, qk_b(0, sb0), unroll=3)

    @pl.when(t == 0)
    def _init_kv_a():
        copies[3].wait()
        xa = xa_ref[...]
        nt = (((1,), (1,)), ((), ()))
        k = lax.dot_general(xa, wkt_ref[...], nt, preferred_element_type=f32)
        vt = lax.dot_general(wvt_ref[...], xa, nt, preferred_element_type=f32)
        ka_ref[...] = k.astype(bf16)
        vta_ref[...] = vt.astype(bf16)
        copies[4].wait()

    ms1 = stage_b(NG - 1, sb1, NG - 2, sb0, ms)
    pv_b(NG - 1, sb1, ms1)

    xa_t = xa_ref[pl.ds(row0, TQ), :]
    q = jnp.dot(xa_t, wq_ref[...], preferred_element_type=f32) * QSCALE
    qt_ref[...] = q.T.astype(bf16)

    def qk_a(h, buf):
        r0 = pl.multiple_of(h * DH, DH)
        qh = qt_ref[pl.ds(r0, DH), :]
        m8 = None
        for c in range(S // CQ):
            st = jnp.dot(ka_ref[c * CQ:(c + 1) * CQ, :], qh, preferred_element_type=f32)
            buf[c * CQ:(c + 1) * CQ, :] = st
            mc = jnp.max(st.reshape(CQ // 8, 8, TQ), axis=0)
            m8 = mc if m8 is None else jnp.maximum(m8, mc)
        return jnp.max(m8, axis=0, keepdims=True)

    def pv_a(h, buf, m):
        r0 = pl.multiple_of(h * DH, DH)
        l8 = None
        acc = None
        for c in range(NC):
            p = jnp.exp2(buf[c * CK:(c + 1) * CK, :] - m)
            lc = jnp.sum(p.reshape(CK // 8, 8, TQ), axis=0)
            l8 = lc if l8 is None else l8 + lc
            d = jnp.dot(vta_ref[:, c * CK:(c + 1) * CK], p.astype(bf16),
                        preferred_element_type=f32)
            acc = d if acc is None else acc + d
        ota_ref[pl.ds(r0, DH), :] = acc / jnp.sum(l8, axis=0, keepdims=True)

    def stage_a(hq, bufq, hp, bufp, m):
        rq = pl.multiple_of(hq * DH, DH)
        rp = pl.multiple_of(hp * DH, DH)
        qh = qt_ref[pl.ds(rq, DH), :]
        m8 = None
        l8 = None
        acc = None
        for c in range(NC):
            st = jnp.dot(ka_ref[c * CK:(c + 1) * CK, :], qh, preferred_element_type=f32)
            bufq[c * CK:(c + 1) * CK, :] = st
            mc = jnp.max(st.reshape(CK // 8, 8, TQ), axis=0)
            m8 = mc if m8 is None else jnp.maximum(m8, mc)
            p = jnp.exp2(bufp[c * CK:(c + 1) * CK, :] - m)
            lc = jnp.sum(p.reshape(CK // 8, 8, TQ), axis=0)
            l8 = lc if l8 is None else l8 + lc
            d = jnp.dot(vta_ref[:, c * CK:(c + 1) * CK], p.astype(bf16),
                        preferred_element_type=f32)
            acc = d if acc is None else acc + d
        ota_ref[pl.ds(rp, DH), :] = acc / jnp.sum(l8, axis=0, keepdims=True)
        return jnp.max(m8, axis=0, keepdims=True)

    def body_a(i, m):
        h = 2 * i
        m1 = stage_a(h + 1, sa1, h, sa0, m)
        m2 = stage_a(h + 2, sa0, h + 1, sa1, m1)
        return m2

    m = lax.fori_loop(0, H // 2 - 1, body_a, qk_a(0, sa0))

    @pl.when(t == 0)
    def _wait_wo():
        copies[5].wait()
        copies[6].wait()

    m1 = stage_a(H - 1, sa1, H - 2, sa0, m)
    pv_a(H - 1, sa1, m1)

    ob = otb_ref[...].T.astype(bf16)
    o_ref[:, D:2 * D] = jnp.dot(ob, wob_ref[...], preferred_element_type=f32).astype(o_ref.dtype)
    oa = ota_ref[...].T.astype(bf16)
    o_ref[:, 0:D] = jnp.dot(oa, woa_ref[...], preferred_element_type=f32).astype(o_ref.dtype)


@jax.jit
def pallas_concat_heads__grouped_kv_mqa__sliding_block__prompt_kernel(
    A_x: jax.Array,
    A_wq: jax.Array,
    A_wk: jax.Array,
    A_wv: jax.Array,
    A_wo: jax.Array,
    B_x: jax.Array,
    B_wqkv: jax.Array,
    B_wo: jax.Array,
):
    xa = A_x.reshape(S, D)
    xb = B_x.reshape(S, D)
    bf16 = jnp.bfloat16
    f32 = jnp.float32
    const = lambda shape: pl.BlockSpec(shape, lambda t: (0, 0))
    hbm = pl.BlockSpec(memory_space=pl.ANY)
    out = pl.pallas_call(
        _kernel,
        grid=(NT,),
        in_specs=[
            hbm, hbm, const((DH, D)), const((DH, D)), hbm,
            pl.BlockSpec((TQ, D), lambda t: (t, 0)), hbm, hbm,
        ],
        out_specs=pl.BlockSpec((TQ, 2 * D), lambda t: (t, 0)),
        out_shape=jax.ShapeDtypeStruct((S, 2 * D), bf16),
        scratch_shapes=[
            pltpu.VMEM((S, D), bf16),
            pltpu.VMEM((D, D), bf16),
            pltpu.VMEM((D, D), bf16),
            pltpu.VMEM((D, 3 * D), bf16),
            pltpu.VMEM((D, D), bf16),
            pltpu.SemaphoreType.DMA((7,)),
            pltpu.VMEM((S, DH), bf16),
            pltpu.VMEM((DH, S), bf16),
            pltpu.VMEM((D, TQ), bf16),
            pltpu.VMEM((D, TQ), f32),
            pltpu.VMEM((D, TQ), f32),
            pltpu.VMEM((S, D), bf16),
            pltpu.VMEM((D, S), bf16),
            pltpu.VMEM((S, TQ), f32),
            pltpu.VMEM((S, TQ), f32),
            pltpu.VMEM((4, D, TQ), bf16),
            pltpu.VMEM((NSUB, KW, 128), f32),
            pltpu.VMEM((NSUB * 4, KW, 128), f32),
            pltpu.VMEM((NSUB * 4, KW, 128), f32),
        ],
        compiler_params=pltpu.CompilerParams(
            dimension_semantics=("arbitrary",),
            vmem_limit_bytes=100 * 1024 * 1024),
    )(xa, A_wq, A_wk.T, A_wv.T, A_wo, xb, B_wqkv, B_wo)
    return out.reshape(1, S, 2 * D)
```

```python
import jax
import jax.numpy as jnp
from jax import lax
import jax.experimental.pallas as pl
import jax.experimental.pallas.tpu as pltpu

S = 2048
D = 1024
H = 32
DH = 32
W = 256
TQ = 256
NT = S // TQ
LOG2E = 1.4426950408889634
QSCALE = (DH ** -0.5) * LOG2E
CK = 256
NC = S // CK
KW = 384
NSUB = TQ // 128
NG = H // 4
NEG = -1e30


def _kernel(xa_hbm, wq_hbm, wkt_ref, wvt_ref, woa_hbm, xb_hbm, wqkv_hbm, wob_hbm,
            o_ref,
            xa_ref, xb_ref, wq_ref, woa_ref, wqkv_ref, wob_ref, sems,
            ka_ref, vta_ref, qt_ref, ota_ref, otb_ref, kb_ref, vtb_ref, sa0, sa1, qm_ref,
            bias_ref, sb0, sb1, ob_ref):
    t = pl.program_id(0)
    f32 = jnp.float32
    bf16 = jnp.bfloat16

    copies = [
        pltpu.make_async_copy(xb_hbm.at[0:TQ, :], xb_ref.at[0:TQ, :], sems.at[0]),
        pltpu.make_async_copy(wqkv_hbm.at[:, 0:D], wqkv_ref.at[:, 0:D], sems.at[1]),
        pltpu.make_async_copy(wqkv_hbm.at[:, D:2 * D], wqkv_ref.at[:, D:2 * D], sems.at[2]),
        pltpu.make_async_copy(wqkv_hbm.at[:, 2 * D:3 * D], wqkv_ref.at[:, 2 * D:3 * D], sems.at[3]),
        pltpu.make_async_copy(xa_hbm, xa_ref, sems.at[4]),
        pltpu.make_async_copy(wq_hbm, wq_ref, sems.at[5]),
        pltpu.make_async_copy(wob_hbm, wob_ref, sems.at[6]),
        pltpu.make_async_copy(xb_hbm.at[TQ:S, :], xb_ref.at[TQ:S, :], sems.at[7]),
        pltpu.make_async_copy(woa_hbm, woa_ref, sems.at[8]),
    ]

    row0 = pl.multiple_of(t * TQ, TQ)
    rowj = (lax.broadcasted_iota(jnp.int32, (128, TQ), 0) // DH) % 4

    def proj_q(r, i):
        c0 = pl.multiple_of(i * 128, 128)
        y = jnp.dot(xb_ref[pl.ds(r, TQ), :], wqkv_ref[:, pl.ds(c0, 128)],
                    preferred_element_type=f32) * QSCALE
        yt = y.T
        for j in range(4):
            qm_ref[j, pl.ds(c0, 128), :] = jnp.where(rowj == j, yt, 0.0).astype(bf16)

    def proj_k(r, i):
        c0 = pl.multiple_of(i * 128, 128)
        y = jnp.dot(xb_ref[pl.ds(r, TQ), :], wqkv_ref[:, pl.ds(D + c0, 128)],
                    preferred_element_type=f32)
        kb_ref[pl.ds(r, TQ), pl.ds(c0, 128)] = y.astype(bf16)

    def proj_v(r, i):
        c0 = pl.multiple_of(i * 128, 128)
        y = jnp.dot(xb_ref[pl.ds(r, TQ), :], wqkv_ref[:, pl.ds(2 * D + c0, 128)],
                    preferred_element_type=f32)
        vtb_ref[pl.ds(c0, 128), pl.ds(r, TQ)] = y.T.astype(bf16)

    @pl.when(t == 0)
    def _start():
        for c in copies:
            c.start()
        kb_ref[TQ:KW, :] = jnp.zeros((KW - TQ, D), bf16)
        vtb_ref[:, TQ:KW] = jnp.zeros((D, KW - TQ), bf16)
        copies[0].wait()
        copies[1].wait()
        for i in range(8):
            proj_q(0, i)
        copies[2].wait()
        for i in range(8):
            proj_k(0, i)
        copies[3].wait()
        for i in range(8):
            proj_v(0, i)

    k0s = []
    for sub in range(NSUB):
        q0 = row0 + sub * 128
        k0 = pl.multiple_of(jnp.maximum(q0 - W, 0), 128)
        k0s.append(k0)
        kpos = k0 + lax.broadcasted_iota(jnp.int32, (KW, 128), 0)
        qpos = q0 + lax.broadcasted_iota(jnp.int32, (KW, 128), 1)
        d = qpos - kpos
        bias_ref[sub] = jnp.where((d >= 0) & (d < W), 0.0, NEG).astype(f32)

    def stage_b(gq, bufq, gp, bufp, msp):
        ms = []
        for sub in range(NSUB):
            if gq is not None:
                cq = pl.multiple_of(gq * 128, 128)
                kg = kb_ref[pl.ds(k0s[sub], KW), pl.ds(cq, 128)]
            if gp is not None:
                cp = pl.multiple_of(gp * 128, 128)
                vtg = vtb_ref[pl.ds(cp, 128), pl.ds(k0s[sub], KW)]
            for j in range(4):
                if gq is not None:
                    qm = qm_ref[j, pl.ds(cq, 128), sub * 128:(sub + 1) * 128]
                    st = jnp.dot(kg, qm, preferred_element_type=f32) + bias_ref[sub]
                    bufq[sub * 4 + j] = st
                    ms.append(jnp.max(st, axis=0, keepdims=True))
                if gp is not None:
                    p = jnp.exp2(bufp[sub * 4 + j] - msp[sub * 4 + j])
                    l = jnp.sum(p, axis=0, keepdims=True)
                    ot = jnp.dot(vtg[j * DH:(j + 1) * DH, :], p.astype(bf16),
                                 preferred_element_type=f32)
                    otb_ref[pl.ds(cp + j * DH, DH), sub * 128:(sub + 1) * 128] = ot / l
        return tuple(ms)

    ms = stage_b(0, sb0, None, None, None)
    for i in range(NG // 2 - 1):
        g = 2 * i
        ms = stage_b(g + 1, sb1, g, sb0, ms)
        ms = stage_b(g + 2, sb0, g + 1, sb1, ms)

    @pl.when(t == 0)
    def _init_kv_a():
        copies[4].wait()
        xa = xa_ref[...]
        nt = (((1,), (1,)), ((), ()))
        k = lax.dot_general(xa, wkt_ref[...], nt, preferred_element_type=f32)
        vt = lax.dot_general(wvt_ref[...], xa, nt, preferred_element_type=f32)
        ka_ref[...] = k.astype(bf16)
        vta_ref[...] = vt.astype(bf16)
        copies[5].wait()
        copies[6].wait()
        copies[7].wait()

    ms = stage_b(NG - 1, sb1, NG - 2, sb0, ms)
    stage_b(None, None, NG - 1, sb1, ms)
    ob_ref[...] = otb_ref[...].T.astype(bf16)

    def proj_ob(_, i):
        c0 = pl.multiple_of(i * 128, 128)
        y = jnp.dot(ob_ref[...], wob_ref[:, pl.ds(c0, 128)], preferred_element_type=f32)
        o_ref[:, pl.ds(D + c0, 128)] = y.astype(o_ref.dtype)

    xa_t = xa_ref[pl.ds(row0, TQ), :]
    q = jnp.dot(xa_t, wq_ref[...], preferred_element_type=f32) * QSCALE
    qt_ref[...] = q.T.astype(bf16)

    def stage_a(hq, bufq, hp, bufp, m, extra=None):
        if hq is not None:
            rq = pl.multiple_of(hq * DH, DH)
            qh = qt_ref[pl.ds(rq, DH), :]
        m8 = None
        l8 = None
        acc = None
        for c in range(NC):
            if hq is not None:
                st = jnp.dot(ka_ref[c * CK:(c + 1) * CK, :], qh, preferred_element_type=f32)
                bufq[c * CK:(c + 1) * CK, :] = st
                mc = jnp.max(st.reshape(CK // 8, 8, TQ), axis=0)
                m8 = mc if m8 is None else jnp.maximum(m8, mc)
            if hp is not None:
                p = jnp.exp2(bufp[c * CK:(c + 1) * CK, :] - m)
                lc = jnp.sum(p.reshape(CK // 8, 8, TQ), axis=0)
                l8 = lc if l8 is None else l8 + lc
                d = jnp.dot(vta_ref[:, c * CK:(c + 1) * CK], p.astype(bf16),
                            preferred_element_type=f32)
                acc = d if acc is None else acc + d
            if extra is not None and c == 0:
                extra()
        if hp is not None:
            rp = pl.multiple_of(hp * DH, DH)
            ota_ref[pl.ds(rp, DH), :] = acc / jnp.sum(l8, axis=0, keepdims=True)
        if hq is not None:
            return jnp.max(m8, axis=0, keepdims=True)

    rnext = pl.multiple_of(jnp.minimum(row0 + TQ, S - TQ), TQ)

    def make_body(base, proj):
        def body(i, m):
            h = 2 * i
            if proj is None:
                e1 = e2 = None
            else:
                e1 = lambda: proj(rnext, 2 * (i - base))
                e2 = lambda: proj(rnext, 2 * (i - base) + 1)
            m1 = stage_a(h + 1, sa1, h, sa0, m, e1)
            return stage_a(h + 2, sa0, h + 1, sa1, m1, e2)
        return body

    m = stage_a(0, sa0, None, None, None)
    NI = H // 2 - 1

    def with_proj(m):
        m = lax.fori_loop(0, 4, make_body(0, proj_q), m)
        m = lax.fori_loop(4, 8, make_body(4, proj_k), m)
        return lax.fori_loop(8, 12, make_body(8, proj_v), m)

    def without_proj(m):
        return lax.fori_loop(0, 12, make_body(0, None), m)

    m = lax.cond(t < NT - 1, with_proj, without_proj, m)
    m = lax.fori_loop(12, NI, make_body(12, proj_ob), m)

    @pl.when(t == 0)
    def _wait_wo():
        copies[8].wait()

    m1 = stage_a(H - 1, sa1, H - 2, sa0, m, lambda: proj_ob(None, 6))
    stage_a(None, None, H - 1, sa1, m1, lambda: proj_ob(None, 7))

    oa = ota_ref[...].T.astype(bf16)
    o_ref[:, 0:D] = jnp.dot(oa, woa_ref[...], preferred_element_type=f32).astype(o_ref.dtype)


@jax.jit
def pallas_concat_heads__grouped_kv_mqa__sliding_block__prompt_kernel(
    A_x: jax.Array,
    A_wq: jax.Array,
    A_wk: jax.Array,
    A_wv: jax.Array,
    A_wo: jax.Array,
    B_x: jax.Array,
    B_wqkv: jax.Array,
    B_wo: jax.Array,
):
    xa = A_x.reshape(S, D)
    xb = B_x.reshape(S, D)
    bf16 = jnp.bfloat16
    f32 = jnp.float32
    const = lambda shape: pl.BlockSpec(shape, lambda t: (0, 0))
    hbm = pl.BlockSpec(memory_space=pl.ANY)
    out = pl.pallas_call(
        _kernel,
        grid=(NT,),
        in_specs=[hbm, hbm, const((DH, D)), const((DH, D)), hbm, hbm, hbm, hbm],
        out_specs=pl.BlockSpec((TQ, 2 * D), lambda t: (t, 0)),
        out_shape=jax.ShapeDtypeStruct((S, 2 * D), bf16),
        scratch_shapes=[
            pltpu.VMEM((S, D), bf16),
            pltpu.VMEM((S, D), bf16),
            pltpu.VMEM((D, D), bf16),
            pltpu.VMEM((D, D), bf16),
            pltpu.VMEM((D, 3 * D), bf16),
            pltpu.VMEM((D, D), bf16),
            pltpu.SemaphoreType.DMA((9,)),
            pltpu.VMEM((S, DH), bf16),
            pltpu.VMEM((DH, S), bf16),
            pltpu.VMEM((D, TQ), bf16),
            pltpu.VMEM((D, TQ), f32),
            pltpu.VMEM((D, TQ), f32),
            pltpu.VMEM((S, D), bf16),
            pltpu.VMEM((D, S), bf16),
            pltpu.VMEM((S, TQ), f32),
            pltpu.VMEM((S, TQ), f32),
            pltpu.VMEM((4, D, TQ), bf16),
            pltpu.VMEM((NSUB, KW, 128), f32),
            pltpu.VMEM((NSUB * 4, KW, 128), f32),
            pltpu.VMEM((NSUB * 4, KW, 128), f32),
            pltpu.VMEM((TQ, D), bf16),
        ],
        compiler_params=pltpu.CompilerParams(
            dimension_semantics=("arbitrary",),
            vmem_limit_bytes=100 * 1024 * 1024),
    )(xa, A_wq, A_wk.T, A_wv.T, A_wo, xb, B_wqkv, B_wo)
    return out.reshape(1, S, 2 * D)
```
